```python
import os as _os
_os.environ.setdefault("JAX_PLATFORMS", "cpu")
import jax
import jax.numpy as jnp

def _softmax(x, axis=-1):
    return jax.nn.softmax(x, axis=axis)
def _gelu(x):
    return jax.nn.gelu(x, approximate=True)
def _silu(x):
    return jax.nn.silu(x)
def _sigmoid(x):
    return jax.nn.sigmoid(x)
def _layernorm(x, axis=-1, eps=1e-5):
    m = jnp.mean(x, axis=axis, keepdims=True)
    v = jnp.var(x, axis=axis, keepdims=True)
    return (x - m) / jnp.sqrt(v + eps)
def _scatter_add(tgt, idx, src, axis=0):
    return tgt.at[idx].add(src)
def _segment_sum(src, seg, n):
    return jax.ops.segment_sum(src, seg, n)
class _Rng:
    def __init__(self, key):
        self._k = key
    def _next(self):
        self._k, sub = jax.random.split(self._k)
        return sub
    def normal(self, shape):
        return jax.random.normal(self._next(), shape, dtype=jnp.bfloat16)
    def randint(self, lo, hi, shape):
        return jax.random.randint(self._next(), shape, lo, hi, dtype=jnp.int32)
    def uniform(self, shape, lo=0.0, hi=1.0):
        return jax.random.uniform(self._next(), shape, jnp.bfloat16, lo, hi)
    def permutation(self, n):
        return jax.random.permutation(self._next(), n)


kernel_name = 'sequential_preLN__sliding_block__swiglu_ffn__prompt'

def setup_inputs():
    _rng = _Rng(jax.random.key(int.from_bytes(__import__("os").urandom(4), "little")))
    _w = (lambda a: (lambda t: t.astype(jnp.bfloat16) if jnp.issubdtype(t.dtype, jnp.floating) else t)(jnp.asarray(a)))
    def _A_setup():
        B, S, D = 1, 2048, 512
        return {
            "x": _w((lambda *s: _rng.normal(s) * 0.05)(B, S, D)),
            "wqkv": _w((lambda *s: _rng.normal(s) * 0.05)(D, 3 * D)),
            "wo": _w((lambda *s: _rng.normal(s) * 0.05)(D, D)),
        }
    _A_in = _A_setup()

    def _B_setup():
        B, S, D, F = 1, 2048, 512, 1792
        return {
            "x": _w((lambda *s: _rng.normal(s) * 0.05)(B, S, D)),
            "w_gate": _w((lambda *s: _rng.normal(s) * 0.05)(D, F)),
            "w_up": _w((lambda *s: _rng.normal(s) * 0.05)(D, F)),
            "w_down": _w((lambda *s: _rng.normal(s) * 0.05)(F, D)),
        }
    _B_in = _B_setup()

    return {
        "A_x": _A_in["x"],
        "A_wqkv": _A_in["wqkv"],
        "A_wo": _A_in["wo"],
        "B_x": _B_in["x"],
        "B_w_gate": _B_in["w_gate"],
        "B_w_up": _B_in["w_up"],
        "B_w_down": _B_in["w_down"],
    }

def reference(A_x, A_wqkv, A_wo, B_x, B_w_gate, B_w_up, B_w_down):
    def _A_ref(x, wqkv, wo):
        B, S, D = x.shape
        H = 32; Dh = D // H; W = 256
        qkv = (lambda x, *d: x.transpose(*d))((x @ wqkv).reshape(B, S, 3, H, Dh), 2, 0, 3, 1, 4)
        q, k, v = qkv[0], qkv[1], qkv[2]
        scores = jnp.einsum("bhqd,bhkd->bhqk", q, k) * (Dh ** -0.5)
        idx = jnp.arange(S)
        mask = (idx[:, None] - idx[None, :] >= 0) & (idx[:, None] - idx[None, :] < W)
        scores = jnp.where(mask[None, None], scores, -1e9)
        p = _softmax(scores, axis=-1)
        o = jnp.einsum("bhqk,bhkd->bhqd", p, v)
        return (lambda x, *d: x.transpose(*d))(o, 0, 2, 1, 3).reshape(B, S, D) @ wo

    def _B_ref(x, w_gate, w_up, w_down):
        g = _silu(x @ w_gate)
        u = x @ w_up
        return (g * u) @ w_down

    x = A_x
    h = x + _A_ref(_layernorm(x, axis=-1), A_wqkv, A_wo)
    h2 = h + _B_ref(_layernorm(h, axis=-1), B_w_gate, B_w_up, B_w_down)
    return h2
```

```python
import numpy as np
import jax
import jax.numpy as jnp
from jax import lax
import jax.experimental.pallas as pl
import jax.experimental.pallas.tpu as pltpu

S, D, H, DH, W, F = 2048, 512, 32, 16, 256, 1792
EPS = 1e-5
QSCALE = float(DH ** -0.5 * np.log2(np.e))
NEG = -1e30
BF, F32, I32 = jnp.bfloat16, jnp.float32, jnp.int32
NT = (((1,), (1,)), ((), ()))


def _ln(x):
    m = jnp.mean(x, axis=-1, keepdims=True)
    xc = x - m
    v = jnp.mean(xc * xc, axis=-1, keepdims=True)
    return xc * lax.rsqrt(v + EPS)


def _chain(op, xs, n=4):
    accs = list(xs[:n])
    for t, v in enumerate(xs[n:]):
        accs[t % n] = op(accs[t % n], v)
    while len(accs) > 1:
        accs = [op(accs[i], accs[i + 1]) if i + 1 < len(accs) else accs[i] for i in range(0, len(accs), 2)]
    return accs[0]


def _rows8(x):
    return [x[r:r + 8] for r in range(0, x.shape[0], 8)]


def _recip(l):
    r = pl.reciprocal(l, approx=True)
    return r * (2.0 - l * r)


LEFT = ((0, 1, 3), (2, 1, 3), (0,), (3,), (0, 1, 1), (2, -1, 0), (1, -1, 3))
RIGHT = ((0, 1, 3), (0,), (1, -1, 3), (2, -1, 0), (3,), (0, 1, 1), (2, 1, 3))


def _operand(term, quadrants):
    if len(term) == 1:
        return quadrants[term[0]]
    a, sign, b = term
    return quadrants[a] + quadrants[b] if sign > 0 else quadrants[a] - quadrants[b]


def _two_levels(table, q):
    for outer in table:
        inner = [_operand(outer, (q[r][c], q[r][2 + c], q[2 + r][c], q[2 + r][2 + c]))
                 for r in range(2) for c in range(2)]
        for term in table:
            yield _operand(term, inner)


def _widen(block):
    return block.astype(F32)


def _narrow(v):
    return pltpu.bitcast(v.astype(BF), I32)


def _bcomb(*quadrants):
    wide = [_widen(v) for v in quadrants]
    return [pltpu.bitcast(quadrants[term[0]], I32) if len(term) == 1 else _narrow(_operand(term, wide))
            for term in RIGHT]


def _combine(m):
    m2, m4, m3, m5 = m(1), m(3), m(2), m(4)
    c21, c12, c22, c11 = m2 + m4, m3 + m5, m3 - m2, m4 - m5
    m1 = m(0)
    return (c11 + m1) + m(6), c12, c21, (c22 + m1) + m(5)


class _Pool:
    def __init__(self, refs, zero):
        self.refs, self.zero, self.free = refs, zero, list(range(len(refs)))

    def put(self, value):
        slot = self.free.pop(0)
        self.refs[slot][0:value.shape[0], :] = value
        return slot, value.shape[0]

    def get(self, handle):
        return self.refs[handle[0]][pl.ds(self.zero, handle[1]), :]

    def pop(self, handle):
        self.free.append(handle[0])
        return self.get(handle)


def _strassen(mm, cost, done):
    c = {}
    def t0():
        m2, m4 = mm(1), mm(3)
        c["m2"], c["m4"] = m2, m4
        done(2, m2 + m4)
    def t1():
        m3, m5 = mm(2), mm(4)
        c[22], c[11] = m3 - c.pop("m2"), c.pop("m4") - m5
        done(1, m3 + m5)
    def t2():
        m1 = mm(0)
        done(3, (c.pop(22) + m1) + mm(5))
        done(0, (c.pop(11) + m1) + mm(6))
    return [(2 * cost, 0, t0), (2 * cost, 0, t1), (3 * cost, 0, t2)]


def _swap_blocks(v, lane):
    lo64 = lane < 64
    w = [None] * 4
    for c in (0, 1):
        r = pltpu.roll(jnp.where(lo64, v[c + 2], v[c]), 64, 1)
        w[c], w[c + 2] = jnp.where(lo64, v[c], r), jnp.where(lo64, r, v[c + 2])
    lo32 = (lane & 32) == 0
    out = [None] * 4
    for c in (0, 2):
        out[c] = jnp.where(lo32, w[c], pltpu.roll(w[c + 1], 32, 1))
        out[c + 1] = jnp.where(lo32, pltpu.roll(w[c], 96, 1), w[c + 1])
    return out


class _Packed:
    def __init__(self, ref):
        self.ref = ref

    def _index(self, idx):
        idx = list(idx) if isinstance(idx, tuple) else [idx]
        idx += [slice(None)] * (len(self.ref.shape) - len(idx))
        r = idx[-2]
        if r != slice(None):
            assert r.start % 16 == 0 and r.stop % 16 == 0
            idx[-2] = slice(r.start // 2, r.stop // 2)
        return tuple(idx)

    def __getitem__(self, idx):
        return pltpu.bitcast(self.ref[self._index(idx)], BF)

    def __setitem__(self, idx, value):
        self.ref[self._index(idx)] = value if value.dtype == I32 else pltpu.bitcast(value, I32)


def _build():
    pos = (0, 0.3, 0.6, 0.8, 1.0, 1.2, 1.45, 1.45, 1.45, 1.45)
    span, span0, span1 = (0.03, 1.0), 0.25, (0.03, 0.34)
    nq0, ogrp, gate = 3, (5, 7, 8), (6, 1)
    lag, lnlag, pdel, look, wdn, RC, NS = 48, 128, 300, 1, 2, 64, 32
    flags = {"XLA_TPU_EVENLY_DISTRIBUTE_CRITICAL_NODES": True}
    T, QN, WN, DN, PR, GR = 256, 128, 128, 128, 16, 16
    NB, NL, TH, TQ, HD, HF = S // T, T // 128, T // 2, T // 4, D // 2, F // 2
    dot = lambda a, b: jnp.dot(a, b, preferred_element_type=F32)
    dnt = lambda a, b: lax.dot_general(a, b, NT, preferred_element_type=F32)

    def kernel(x_h, wqkv_h, wo_h, wg_h, wu_h, wd_h, o_h,
               x_v, wq_d, wk_d, wv_d, wo_d, wg_d, wu_d, wd_d,
               wvT, q_s, k_s, vT_s, oT_s, h_s, hn_s, a_s, xn0_s, xn1_s, oc_s, o_v,
               wsem, xsem, osem, fence, *tiles):
        wvT, q_s, k_s, vT_s, oT_s, hn_s, a_s, oc_s, *xn_s = map(
            _Packed, (wvT, q_s, k_s, vT_s, oT_s, hn_s, a_s, oc_s, xn0_s, xn1_s))
        zero = pl.multiple_of(jnp.min(lax.broadcasted_iota(I32, (8, 128), 1)), 8)
        spool = _Pool(tiles[:NS], zero)
        parts = list(map(_Packed, tiles[NS:]))
        wqk, wo, wgu, wd = parts[0:4], parts[4:6], parts[6:13], parts[13:15]
        fresh = lambda is_fresh: zero if is_fresh else 0
        xb = (0, 2 * T, (nq0 + 2) * T, S)
        ob = (0,) + tuple(T * n for n in ogrp)
        copies = lambda src, dst, bounds, sem: [
            pltpu.make_async_copy(src.at[lo:hi], dst.at[lo:hi], sem.at[n])
            for n, (lo, hi) in enumerate(zip(bounds, bounds[1:]))]
        x_cp, o_cp = copies(x_h, x_v, xb, xsem), copies(o_v, o_h, ob, osem)
        w_cp = [pltpu.make_async_copy(s, d, wsem.at[n]) for n, (s, d) in enumerate(
            [(wqkv_h.at[:, 0:D], wq_d), (wqkv_h.at[:, D:2 * D], wk_d), (wqkv_h.at[:, 2 * D:3 * D], wv_d),
             (wo_h, wo_d), (wg_h, wg_d), (wu_h, wu_d), (wd_h, wd_d)])]

        def start_in_order(cps):
            for c in cps:
                c.start()
                pl.semaphore_signal(fence)
                pl.semaphore_wait(fence)

        def wait_all(cps):
            for c in cps:
                c.wait()

        def acomb_tasks(dst, rows, delay):
            def f(r):
                top, bot = rows(r, RC), rows(TH + r, RC)
                for j, term in enumerate(LEFT):
                    dst[j, r:r + RC] = _narrow(_operand(term, (top[:, :HD], top[:, HD:], bot[:, :HD], bot[:, HD:])))
            return [(0, delay + lnlag * (r // RC), lambda r=r: f(r)) for r in range(0, TH, RC)]

        def put_bcomb(dst, left, lc, right, rc, kh, lo=0, hi=None):
            for r in range(lo, kh if hi is None else hi, PR):
                top, bot = slice(r, r + PR), slice(kh + r, kh + r + PR)
                for j, c in enumerate(_bcomb(left[top, lc], right[top, rc], left[bot, lc], right[bot, rc])):
                    dst[j, top] = c

        def prep_qk(c):
            cs = slice(c, c + QN)
            put_bcomb(wqk[c // 128], wq_d, cs, wk_d, cs, HD)

        def prep_v():
            wt = wv_d[...].T
            for r in range(0, HD, PR):
                top, bot = wt[r:r + PR], wt[HD + r:HD + r + PR]
                for j, v in enumerate(_bcomb(top[:, :HD], bot[:, :HD], top[:, HD:], bot[:, HD:])):
                    wvT[j, r:r + PR] = v

        def put_v(i, d0, half, v):
            for j in range(NL // 2):
                vT_s[i * NL + half * (NL // 2) + j, d0:d0 + v.shape[0], :] = v[:, 128 * j:128 * j + 128].astype(BF)

        def qkv_tasks(i):
            slot, r0 = i % 2, i * T
            ln = acomb_tasks(xn_s[i % 2], lambda r, n: _ln(_widen(x_v[r0 + r:r0 + r + n])), 0)
            def qk_piece(c):
                cs = slice(c, c + QN)
                def done(n, v):
                    rs = TH * (n // 2)
                    if n % 2 == 0:
                        q_s[r0 + rs:r0 + rs + TH, cs] = (v * QSCALE).astype(BF)
                    else:
                        k_s[r0 + rs:r0 + rs + TH, cs] = v.astype(BF)
                return _strassen(lambda j: dot(xn_s[i % 2][j], wqk[c // 128][j + fresh(i == 2)]), T * QN // 512, done)
            def v_piece(c):
                return _strassen(lambda j: dnt(wvT[j + fresh(i == 2), c:c + QN, :], xn_s[i % 2][j]), T * QN // 512,
                                 lambda n, v: put_v(i, c + HD * (n % 2), n // 2, v))
            return [ln] + [qk_piece(c) for c in range(0, D, QN)] + [v_piece(c) for c in range(0, HD, QN)]

        def qkv_first():
            start_in_order([x_cp[0]] + w_cp[0:3])
            wait_all(x_cp[:1])
            xn = [_ln(x_v[r:r + T].astype(F32)).astype(BF) for r in (0, T)]
            wait_all(w_cp[:1])
            start_in_order([x_cp[1]] + w_cp[3:6] + [x_cp[2], w_cp[6]])
            for n in range(2):
                q_s[n * T:n * T + T] = (dot(xn[n], wq_d[...]) * QSCALE).astype(BF)
            wait_all(w_cp[1:2])
            for n in range(2):
                k_s[n * T:n * T + T] = dot(xn[n], wk_d[...]).astype(BF)
            wait_all([w_cp[2], x_cp[1]])
            env = {}
            def v_piece(n, c):
                if not env:
                    env["wt"] = wv_d[...].T
                v = dnt(env["wt"][c:c + HD], xn[n])
                for half in range(2):
                    put_v(n, c, half, v[:, TH * half:TH * half + TH])
            return [[(T * HD // 128, 0, lambda n=n, c=c: v_piece(n, c)) for c in (0, HD)] for n in range(2)]

        def attn_tasks(i):
            slot = i % 2
            lane8 = lax.broadcasted_iota(I32, (8, 128), 1)
            hm = [jnp.where((lane8 >> 4) == h, -1, 0) for h in range(8)]
            plane = lax.broadcasted_iota(I32, (32, 128), 1)
            pq = ((plane >> 5) << 4) + (plane & 15)
            row16 = lax.broadcasted_iota(I32, (16, 128), 0)
            lane16 = lax.broadcasted_iota(I32, (16, 128), 1)
            tri16 = row16 > (lane16 & 15)
            tri64 = lax.broadcasted_iota(I32, (64, 128), 0) > pq[0:1]
            even16 = (lane16 & 16) == 0
            lane64 = lax.broadcasted_iota(I32, (64, 128), 1)
            units = [(g, 2 * b + e) for b in range(NL) for g in range(D // 128) for e in range(2)]
            qhs, mids, bands, pts, outs = {}, {}, {}, {}, {}

            def qk_mid(u):
                g, a = units[u]
                q0, gs = i * T + 64 * a, slice(128 * g, 128 * g + 128)
                qi = _rows8(pltpu.bitcast(q_s[q0:q0 + 64, gs], I32))
                qhs[u] = qh = [[r & hm[h] for h in range(8)] for r in qi]
                qm = pltpu.bitcast(jnp.concatenate(
                    [qh[c][2 * p + e] for p in range(4) for c in range(4) for e in range(2)], axis=0), BF)
                m0 = max(q0 - W + 64, 0)
                mids[u] = dnt(k_s[m0:q0, gs], qm) if q0 > m0 else None
                if q0 > m0:
                    mids[u] = [spool.put(mids[u][:, 128 * p:128 * p + 128]) for p in range(4)]

            def qk_band(u):
                g, a = units[u]
                q0, gs = i * T + 64 * a, slice(128 * g, 128 * g + 128)
                raw = []
                for c, qh in enumerate(qhs.pop(u)):
                    qc = pltpu.bitcast(jnp.concatenate(qh, axis=0), BF)
                    kl = k_s[q0:q0 + 16 * c + 16, gs]
                    if q0 < W:
                        s = dnt(kl, qc)
                        parts = [s[0:16 * c], jnp.where(tri16, NEG, s[16 * c:]), jnp.full((48 - 16 * c, 128), NEG, F32)]
                    else:
                        s = dnt(jnp.concatenate([kl, k_s[q0 - W + 16 * c:q0 - W + 64, gs]], axis=0), qc)
                        parts = [s[0:16 * c], jnp.where(tri16, s[16 * c + 16:16 * c + 32], s[16 * c:16 * c + 16]),
                                 s[16 * c + 32:]]
                    raw.append(jnp.concatenate([v for v in parts if v.shape[0]], axis=0))
                bands[u] = [spool.put(v) for v in _swap_blocks(raw, lane64)]

            def sm(u, p):
                g, a = units[u]
                partial = i * T + 64 * a < W
                hs = [bands[u][p]] + ([] if mids[u] is None else [mids[u][p]])
                vs = [v for h in hs for v in _rows8(spool.get(h))]
                m = jnp.max(_chain(jnp.maximum, vs[8:] + vs[:8]), axis=0, keepdims=True)
                vs = [v for h in hs for v in _rows8(spool.pop(h))]
                ps = [jnp.exp2(v - m) for v in vs]
                l = jnp.sum(_chain(jnp.add, ps), axis=0, keepdims=True)
                pg = jnp.concatenate(ps[0:8], axis=0)
                blocks = ps[8:] + [pg] if partial else (
                    [jnp.where(tri64, pg, 0.0)] + ps[8:] + [jnp.where(tri64, 0.0, pg)])
                pt = jnp.concatenate(blocks, axis=0)
                pt = pad(a, partial, pt)
                pts[u, p] = (pt, _recip(l))

            def pad(a, partial, pt):
                zero_rows = jnp.zeros((64, 128), F32)
                blocks = [pt, zero_rows] if a % 2 == 0 else [pt] if partial else [zero_rows, pt]
                return jnp.concatenate(blocks, axis=0).astype(BF)

            def pv(u, p):
                g, a = units[u]
                b, r0 = a // 2, 128 * g + 32 * p
                pt, rl = pts.pop((u, p))
                nt = pt.shape[0] // 128
                vt = jnp.concatenate([vT_s[i * NL + b - nt + 1 + j, r0:r0 + 32, :] for j in range(nt)], axis=1)
                outs[u, p] = dot(vt, pt) * rl
                if a % 2 == 1:
                    ea, eb = outs.pop((u - 1, p)), outs.pop((u, p))
                    h0 = jnp.where(even16, ea[0:16], pltpu.roll(eb[0:16], 16, 1))
                    h1 = jnp.where(even16, pltpu.roll(ea[16:32], 112, 1), eb[16:32])
                    oT_s[slot, r0:r0 + 16, 128 * b:128 * b + 128] = h0.astype(BF)
                    oT_s[slot, r0 + 16:r0 + 32, 128 * b:128 * b + 128] = h1.astype(BF)

            tasks = []
            for u in range(len(units)):
                tasks += [(u + pos[0], lambda u=u: qk_mid(u)), (u + pos[1], lambda u=u: qk_band(u))]
                for p in range(4):
                    tasks += [(u + pos[2 + p], lambda u=u, p=p: sm(u, p)), (u + pos[6 + p], lambda u=u, p=p: pv(u, p))]
            return [(t / len(units), f) for t, f in tasks]

        def prep_wo(c):
            put_bcomb(wo[c // 128], wo_d, slice(c, c + WN), wo_d, slice(HD + c, HD + c + WN), HD)
        def prep_gu(c, r0):
            for r in range(r0, r0 + GR, PR):
                blocks = [[_widen(w[128 * n + r:128 * n + r + PR, c + HF * e:c + HF * e + 128])
                           for w in (wg_d, wu_d) for e in range(2)] for n in range(4)]
                for j, v in enumerate(_two_levels(RIGHT, blocks)):
                    wgu[c // 128][j, r:r + PR] = _narrow(v)

        def prep_dn(c, r):
            put_bcomb(wd[c // 128], wd_d, slice(c, c + DN), wd_d, slice(HD + c, HD + c + DN), HF, r, r + 128)

        def ahead(preps, pieces):
            preps = [[(0, pdel * k / len(p) if n >= look else 0, f) for k, f in enumerate(p)] for n, p in enumerate(preps)]
            out = [[t for p in preps[:look] for t in p]] + [[] for _ in pieces[1:]]
            for n, piece in enumerate(pieces):
                out[n] = out[n] + (preps[n + look] if n + look < len(preps) else []) + piece
            return out

        def ffn_tasks(i):
            slot, r0 = i % 2, i * T
            env = {}
            def untranspose(b):
                o = oT_s[slot, :, 128 * b:128 * b + 128].T
                env[b] = jnp.concatenate([o[32 * c + 16 * e:32 * c + 16 * e + 16]
                                          for e in range(2) for c in range(4)], axis=0)
            prep = [(0, 0, lambda b=b: untranspose(b)) for b in range(NL)]
            prep += acomb_tasks(oc_s, lambda r, n: _widen(env[r // 128][r % 128:r % 128 + n]), lnlag)
            def wo_piece(c):
                cc = (slice(c, c + WN), slice(HD + c, HD + c + WN))
                def done(n, v):
                    rs = TH * (n // 2)
                    h_s[slot, cc[n % 2].start // 128, rs:rs + TH] = x_v[r0 + rs:r0 + rs + TH, cc[n % 2]].astype(F32) + v
                return _strassen(lambda j: dot(oc_s[j], wo[c // 128][j + fresh(i == 0)]), T * WN // 512, done)
            def ln2(r):
                def rows(r0):
                    return _ln(jnp.concatenate([h_s[slot, c, r0:r0 + 16] for c in range(4)], axis=1))
                blocks = [[v[:, 128 * c:128 * c + 128] for c in range(4)] for v in map(rows, range(r, T, TQ))]
                for j, v in enumerate(_two_levels(LEFT, blocks)):
                    hn_s[j, r:r + 16] = _narrow(v)
            ln = [(0, lnlag * (1 + r // 16), lambda r=r: ln2(r)) for r in range(0, TQ, 16)]
            def gu_piece(c):
                def left(j, k):
                    lhs = hn_s[7 * j + k]
                    if i == 0 and (j, k) == gate and c + 128 < HF:
                        token = wgu[c // 128 + 1].ref[48 + zero, 0:8, :] & zero
                        words = pltpu.bitcast(lhs, I32)
                        lhs = pltpu.bitcast(jnp.concatenate([words[0:8] | token, words[8:]]), BF)
                    return lhs
                def product(j):
                    c11, c12, c21, c22 = _combine(lambda k: dot(left(j, k), wgu[c // 128][7 * j + k + fresh(i == 0)]))
                    return jnp.concatenate([jnp.concatenate([c11, c12], axis=1), jnp.concatenate([c21, c22], axis=1)])
                def silu(g):
                    hg = 0.5 * g
                    return hg + hg * jnp.tanh(hg)
                held = {}
                def done(n, v):
                    if n == 2:
                        held["s"] = silu(v)
                    elif n == 1:
                        held["u"] = v
                    elif n == 3:
                        held["b"] = held.pop("s") * v
                    else:
                        held["t"] = silu(v) * held.pop("u")
                def put():
                    top, bot = held.pop("t"), held.pop("b")
                    for j, term in enumerate(LEFT):
                        v = _operand(term, (top[:, :128], top[:, 128:], bot[:, :128], bot[:, 128:]))
                        a_s[j, :, c:c + 128] = _narrow(v)
                return _strassen(product, T * 7 // 16, done) + [(0, lag, put)]
            def dn_piece(c):
                cc = (slice(c, c + DN), slice(HD + c, HD + c + DN))
                def done(n, v):
                    rs = TH * (n // 2)
                    o_v[r0 + rs:r0 + rs + TH, cc[n % 2]] = (h_s[slot, cc[n % 2].start // 128, rs:rs + TH] + v).astype(o_v.dtype)
                return _strassen(lambda j: dot(a_s[j], wd[c // 128][j + fresh(i == 0)]), T * DN * 7 // 1024, done)
            cat = lambda ps: [t for p in ps for t in p]
            wos = [wo_piece(c) for c in range(0, HD, WN)]
            gus = [gu_piece(c) for c in range(0, HF, 128)]
            dns = [dn_piece(c) for c in range(0, HD, DN)]
            if i == 0:
                prep = [(0, 0, lambda: wait_all(w_cp[3:] + x_cp[2:]))] + prep
                wos = ahead([[lambda c=c: prep_wo(c)] for c in range(0, HD, WN)], wos)
                pg = [[lambda c=c, r=r: prep_gu(c, r) for r in range(0, 128, GR)] for c in range(0, HF, 128)]
                gus = ahead(pg, gus)
                pd = [lambda c=c, r=r: prep_dn(c, r) for c in range(0, HD, DN) for r in range(0, HF, 128)]
                for n, f in enumerate(pd[:len(pd) // 2]):
                    gus[wdn + n * (len(gus) - wdn) // 7].append((0, 0, f))
                dns[0] = [(0, 0, f) for f in pd[len(pd) // 2:]] + dns[0]
            if i + 1 in ogrp:
                dns[-1] = dns[-1] + [(0, 0, o_cp[ogrp.index(i + 1)].start)]
            return prep, cat(wos) + ln, cat(gus), dns

        def dense_tasks(i):
            ln_of = lambda j: qkv_tasks(j)[0] if j < NB else []
            if i == 0:
                groups = [first[0], ln_of(2) + first[1]]
                for j in range(2, nq0 + 1):
                    pieces = qkv_tasks(j)[1:]
                    if j == 2:
                        pieces = ahead([[lambda c=c: prep_qk(c)] for c in range(0, D, QN)] + [[prep_v]], pieces)
                    groups.append(ln_of(j + 1) + [t for p in pieces for t in p])
            else:
                j = i + nq0
                qt = qkv_tasks(j) if j < NB else [[]] * 7
                f0, f1, f2, f3 = ffn_tasks(i - 1)
                if i == 1:
                    groups = [qt[1] + qt[2], f0 + qt[3], f1 + qt[4] + qt[5], f2 + qt[6]]
                else:
                    dn = ffn_tasks(i - 2)[3]
                    groups = [qt[1] + dn[0][:1], f0 + dn[0][1:] + qt[2], f1 + dn[1] + qt[3],
                              f2 + qt[4] + qt[5] + qt[6]]
                tail = f3[0] + f3[1] if i == NB else []
                groups[-1] = ln_of(j + 1) + groups[-1]
                groups.append(tail)
            total, acc, out = sum(t[0] for g in groups for t in g), 0, []
            for g in groups:
                end = acc + sum(t[0] for t in g)
                for c, delay, f in g:
                    out.append((min(acc + c / 2 + delay, end) / total, f))
                    acc += c
            return out

        def run(tasks):
            for _, f in sorted(tasks, key=lambda t: t[0]):
                f()

        def attn_at(i):
            lo, hi = {0: (span0, 1.0), 1: span1}.get(i, span)
            return [(i + lo + t * (hi - lo), f) for t, f in attn_tasks(i)]

        first = qkv_first()
        tasks = []
        for i in range(NB + 1):
            tasks += [(i + t, f) for t, f in dense_tasks(i)]
            if i < NB:
                tasks += attn_at(i)
        run(tasks)
        wait_all(o_cp)

    def fn(A_x, A_wqkv, A_wo, B_x, B_w_gate, B_w_up, B_w_down):
        anyspec = pl.BlockSpec(memory_space=pl.ANY)
        V = pltpu.VMEM
        P = lambda *sh: V(sh[:-2] + (sh[-2] // 2, sh[-1]), I32)
        out = pl.pallas_call(
            kernel, in_specs=[anyspec] * 6, out_specs=anyspec,
            out_shape=jax.ShapeDtypeStruct((S, D), A_x.dtype),
            scratch_shapes=[V((S, D), BF), V((D, D), BF), V((D, D), BF), V((D, D), BF), V((D, D), BF),
                            V((D, F), BF), V((D, F), BF), V((F, D), BF),
                            P(7, HD, HD),
                            P(S, D), P(S, D), P(S // 128, D, 128), P(2, D, T),
                            V((2, D // 128, T, 128), F32), P(49, TQ, 128), P(7, TH, HF), P(7, TH, HD), P(7, TH, HD), P(7, TH, HD), V((S, D), BF),
                            pltpu.SemaphoreType.DMA((7,)), pltpu.SemaphoreType.DMA((3,)), pltpu.SemaphoreType.DMA((len(ogrp),)),
                            pltpu.SemaphoreType.REGULAR]
            + [V((192, 128), F32)] * NS + [P(7, HD, 128)] * 6 + [P(49, 128, 128)] * 7 + [P(7, HF, 128)] * 2,
            compiler_params=pltpu.CompilerParams(vmem_limit_bytes=100 * 2**20, flags=flags),
            name="fusedblk",
        )(A_x.reshape(S, D), A_wqkv, A_wo, B_w_gate, B_w_up, B_w_down)
        return out.reshape(A_x.shape)
    return fn


@jax.jit
def pallas_sequential_preLN__sliding_block__swiglu_ffn__prompt_kernel(
    A_x: jax.Array,
    A_wqkv: jax.Array,
    A_wo: jax.Array,
    B_x: jax.Array,
    B_w_gate: jax.Array,
    B_w_up: jax.Array,
    B_w_down: jax.Array,
):
    return _build()(A_x, A_wqkv, A_wo, B_x, B_w_gate, B_w_up, B_w_down)
```
